```python
import os as _os
_os.environ.setdefault("JAX_PLATFORMS", "cpu")
import jax
import jax.numpy as jnp

def _softmax(x, axis=-1):
    return jax.nn.softmax(x, axis=axis)
def _gelu(x):
    return jax.nn.gelu(x, approximate=True)
def _silu(x):
    return jax.nn.silu(x)
def _sigmoid(x):
    return jax.nn.sigmoid(x)
def _layernorm(x, axis=-1, eps=1e-5):
    m = jnp.mean(x, axis=axis, keepdims=True)
    v = jnp.var(x, axis=axis, keepdims=True)
    return (x - m) / jnp.sqrt(v + eps)
def _scatter_add(tgt, idx, src, axis=0):
    return tgt.at[idx].add(src)
def _segment_sum(src, seg, n):
    return jax.ops.segment_sum(src, seg, n)
class _Rng:
    def __init__(self, key):
        self._k = key
    def _next(self):
        self._k, sub = jax.random.split(self._k)
        return sub
    def normal(self, shape):
        return jax.random.normal(self._next(), shape, dtype=jnp.bfloat16)
    def randint(self, lo, hi, shape):
        return jax.random.randint(self._next(), shape, lo, hi, dtype=jnp.int32)
    def uniform(self, shape, lo=0.0, hi=1.0):
        return jax.random.uniform(self._next(), shape, jnp.bfloat16, lo, hi)
    def permutation(self, n):
        return jax.random.permutation(self._next(), n)


kernel_name = 'interleave_layers__sliding_local_dilated__mixer_channel_mlp__prompt'

def setup_inputs():
    _rng = _Rng(jax.random.key(int.from_bytes(__import__("os").urandom(4), "little")))
    _w = (lambda a: (lambda t: t.astype(jnp.bfloat16) if jnp.issubdtype(t.dtype, jnp.floating) else t)(jnp.asarray(a)))
    def _A_setup():
        B, S, D = 1, 2048, 512
        return {
            "x": _w((lambda *s: _rng.normal(s) * 0.05)(B, S, D)),
            "wqkv": _w((lambda *s: _rng.normal(s) * 0.05)(D, 3 * D)),
            "wo": _w((lambda *s: _rng.normal(s) * 0.05)(D, D)),
        }
    _A_in = _A_setup()

    def _B_setup():
        B, S, D, F = 1, 2048, 512, 1376
        return {
            "x": _w((lambda *s: _rng.normal(s) * 0.05)(B, S, D)),
            "w1": _w((lambda *s: _rng.normal(s) * 0.4)(D, F) * (D ** -0.5)),
            "b1": _w((lambda *s: _rng.normal(s) * 0.4)(F)),
            "w2": _w((lambda *s: _rng.normal(s) * 0.4)(F, D) * (F ** -0.5)),
            "b2": _w((lambda *s: _rng.normal(s) * 0.4)(D)),
        }
    _B_in = _B_setup()

    return {
        "A_x": _A_in["x"],
        "A_wqkv": _A_in["wqkv"],
        "A_wo": _A_in["wo"],
        "B_x": _B_in["x"],
        "B_w1": _B_in["w1"],
        "B_b1": _B_in["b1"],
        "B_w2": _B_in["w2"],
        "B_b2": _B_in["b2"],
    }

def reference(A_x, A_wqkv, A_wo, B_x, B_w1, B_b1, B_w2, B_b2):
    def _A_ref(x, wqkv, wo):
        B, S, D = x.shape
        H = 32; Dh = D // H
        W, dil = 8, 2
        qkv = (lambda x, *d: x.transpose(*d))((x @ wqkv).reshape(B, S, 3, H, Dh), 2, 0, 3, 1, 4)
        q, k, v = qkv[0], qkv[1], qkv[2]
        scale = Dh ** -0.5
        pos = jnp.arange(S)
        off = jnp.arange(W) * dil
        idx = pos[:, None] - off[None, :]
        mask = idx >= 0
        idx_c = jnp.where(mask, idx, 0).reshape(-1)
        kg = k[:, :, idx_c, :].reshape(B, H, S, W, Dh)
        vg = v[:, :, idx_c, :].reshape(B, H, S, W, Dh)
        logits = jnp.einsum("bhsd,bhswd->bhsw", q, kg) * scale
        logits = jnp.where(mask[None, None, :, :], logits, -1e9)
        attn = _softmax(logits, axis=-1)
        o = jnp.einsum("bhsw,bhswd->bhsd", attn, vg)
        return (lambda x, *d: x.transpose(*d))(o, 0, 2, 1, 3).reshape(B, S, D) @ wo

    def _B_ref(x, w1, b1, w2, b2):
        y = _layernorm(x, axis=-1)
        h = _gelu(jnp.einsum("bsd,df->bsf", y, w1) + b1)
        return jnp.einsum("bsf,fd->bsd", h, w2) + b2

    x = A_x
    x = x + _A_ref(_layernorm(x, axis=-1), A_wqkv, A_wo)
    x = x + _B_ref(_layernorm(x, axis=-1), B_w1, B_b1, B_w2, B_b2)
    x = x + _A_ref(_layernorm(x, axis=-1), A_wqkv, A_wo)
    x = x + _B_ref(_layernorm(x, axis=-1), B_w1, B_b1, B_w2, B_b2)
    return x
```

```python
import functools
import math
import jax
import jax.numpy as jnp
import jax.experimental.pallas as pl
import jax.experimental.pallas.tpu as pltpu

S, D, F = 2048, 512, 1376
H, DH, W, DIL = 32, 16, 8, 2
HALO = 16
EPS = 1e-5
R = 128
T = 2 * R
NSTEP = S // T
RC = 16
f32 = jnp.float32
bf16 = jnp.bfloat16
u32 = jnp.uint32
NT = (((1,), (1,)), ((), ()))
QSCALE = (DH ** -0.5) * math.log2(math.e)
GELU_C1 = math.sqrt(2.0 / math.pi)
GELU_C2 = GELU_C1 * 0.044715
SCOPES = False
GD = 2


def _ln_stats(x):
    m = jnp.mean(x, axis=-1, keepdims=True)
    xc = x - m
    v = jnp.mean(xc * xc, axis=-1, keepdims=True)
    return xc, v


def _ln(x):
    xc, v = _ln_stats(x)
    return xc * jax.lax.rsqrt(v + EPS)


def _ln_ln(x):
    xc, v = _ln_stats(x)
    return xc * jax.lax.rsqrt(v * (1.0 + EPS) + EPS * EPS)


def _pk(x):
    return pltpu.bitcast(x, u32)


def _upk(x):
    return pltpu.bitcast(x, bf16)


def _kernel(x_hbm, wqkv_hbm, wo_hbm, w1t_hbm, b1_hbm, w2_hbm, b2_hbm, o_hbm,
            x_v, o_v, wqkv_v, wo_v, w1t_v, b1_v, w2_v, b2_v,
            wt_p, wo_p, w1_p, w2_p, xn_s, q_s, k_s, v_s, z_s, in_sem, o_sem):
    step = pl.program_id(0)

    copies = {}

    def add_copy(name, src, dst):
        copies[name] = (src, dst, len(copies))

    add_copy("x0", x_hbm.at[pl.ds(0, T), :], x_v.at[pl.ds(0, T), :])
    for t, n in enumerate(("wq", "wk", "wv")):
        add_copy(n, wqkv_hbm.at[:, pl.ds(t * D, D)], wqkv_v.at[:, pl.ds(t * D, D)])
    add_copy("wo", wo_hbm, wo_v)
    add_copy("w1", w1t_hbm, w1t_v)
    add_copy("b1", b1_hbm, b1_v)
    add_copy("b2", b2_hbm, b2_v)
    add_copy("w2", w2_hbm, w2_v)
    add_copy("x1", x_hbm.at[pl.ds(T, T), :], x_v.at[pl.ds(T, T), :])
    add_copy("xr", x_hbm.at[pl.ds(2 * T, S - 2 * T), :], x_v.at[pl.ds(2 * T, S - 2 * T), :])

    def cp(name):
        src, dst, i = copies[name]
        return pltpu.make_async_copy(src, dst, in_sem.at[i])

    def wait(*names):
        if SCOPES:
            with jax.named_scope("wait_" + names[0]):
                for n in names:
                    cp(n).wait()
        else:
            for n in names:
                cp(n).wait()

    def o_copy(i):
        return pltpu.make_async_copy(o_v.at[pl.ds(i * R, R), :], o_hbm.at[pl.ds(i * R, R), :], o_sem.at[i])

    def lmat():
        i = jax.lax.broadcasted_iota(jnp.int32, (128, 128), 0)
        j = jax.lax.broadcasted_iota(jnp.int32, (128, 128), 1)
        return jnp.where(((i >> 3) == (j & 15)) & ((i & 7) == (j >> 4)), 1.0, 0.0).astype(bf16)

    def regroup(outs):
        return jnp.concatenate([outs[hh][d * 8:(d + 1) * 8] for d in range(DH) for hh in range(4)], axis=0)

    def perm_sec(lm, t):
        outs = [jax.lax.dot_general(lm, wqkv_v[:, t * D + hh * 128:t * D + (hh + 1) * 128], NT,
                                    preferred_element_type=f32) for hh in range(4)]
        wt_p[t] = _pk(regroup(outs).astype(bf16))

    def perm_wo(lm):
        outs = [jnp.dot(lm, wo_v[hh * 128:(hh + 1) * 128, :], preferred_element_type=f32) for hh in range(4)]
        wo_p[...] = _pk(regroup(outs).astype(bf16))

    def proj(xn, t):
        return jax.lax.dot_general(xn, _upk(wt_p[t]), NT, preferred_element_type=f32)

    def q_q(xn, l, s):
        q = proj(xn, 0) * QSCALE
        for g in range(4):
            q_s[g, s * R:(s + 1) * R, :] = q[:, g * 128:(g + 1) * 128]

    def q_k(xn, l, s):
        k = proj(xn, 1)
        for g in range(4):
            k_s[l, g, HALO + s * R:HALO + (s + 1) * R, :] = k[:, g * 128:(g + 1) * 128]

    def q_v(xn, l, s):
        v = proj(xn, 2)
        for g in range(4):
            v_s[l, g, HALO + s * R:HALO + (s + 1) * R, :] = v[:, g * 128:(g + 1) * 128]

    def gate(val, dep):
        dz = pltpu.bitcast(dep, u32) & z_s[...]
        return pltpu.bitcast(pltpu.bitcast(val, u32) | dz, val.dtype)

    def attn_o(x, l, s, first):
        rows = []
        deps = []
        for c in range(R // RC):
            r0 = s * R + c * RC
            q = [q_s[g, r0:r0 + RC, :] for g in range(4)]
            logits = []
            for w in range(W):
                off = HALO + r0 - DIL * w
                p = q[0] * k_s[l, 0, off:off + RC, :]
                for g in range(1, 4):
                    p = p + q[g] * k_s[l, g, off:off + RC, :]
                p = p + pltpu.roll(p, 64, 1)
                p = p + pltpu.roll(p, 32, 1)
                if first and r0 < DIL * w:
                    pos = r0 + jax.lax.broadcasted_iota(jnp.int32, (RC, 128), 0)
                    p = jnp.where(pos >= DIL * w, p, -1e9)
                logits.append(p)
            m = logits[0]
            for w in range(1, W):
                m = jnp.maximum(m, logits[w])
            if c >= GD:
                m = gate(m, deps[c - GD])
            e = [jnp.exp2(lg - m) for lg in logits]
            den = e[0]
            for w in range(1, W):
                den = den + e[w]
            inv = pl.reciprocal(den, approx=True)
            inv = inv * (2.0 - den * inv)
            cols = []
            for g in range(4):
                acc = None
                for w in range(W):
                    off = HALO + r0 - DIL * w
                    t = e[w] * v_s[l, g, off:off + RC, :]
                    acc = t if acc is None else acc + t
                cols.append((acc * inv).astype(bf16))
            deps.append(acc)
            rows.append(jnp.concatenate(cols, axis=1))
        if s == 1:
            for g in range(4):
                k_s[l, g, 0:HALO, :] = k_s[l, g, T:T + HALO, :]
                v_s[l, g, 0:HALO, :] = v_s[l, g, T:T + HALO, :]
        a = jnp.concatenate(rows, axis=0)
        return x + jnp.dot(a, _upk(wo_p[...]), preferred_element_type=f32)

    def ln2(x):
        return _ln_ln(x).astype(bf16)

    def up(y, raw=False):
        b1 = b1_v[...].astype(f32).reshape(1, F)
        w = w1t_v[...] if raw else _upk(w1_p[...])
        h = jax.lax.dot_general(y, w, NT, preferred_element_type=f32) + b1
        t = jnp.tanh(h * (GELU_C1 + GELU_C2 * (h * h)))
        return (h + h * t).astype(bf16)

    def down(x, h, raw=False):
        b2 = b2_v[...].astype(f32).reshape(1, D)
        w = w2_v[...] if raw else _upk(w2_p[...])
        return (x + b2) + 0.5 * jnp.dot(h, w, preferred_element_type=f32)

    def ln1(x):
        return _ln(x).astype(bf16)

    def body(first):
        base = 0 if first else pl.multiple_of(step * T, T)
        blk0 = 0 if first else step * 2

        def load_x(s):
            return x_v[pl.ds(base + s * R, R), :].astype(f32)

        def emit(x, s):
            o_v[pl.ds(base + s * R, R), :] = x.astype(bf16)
            o_copy(blk0 + s).start()

        if first:
            for n in copies:
                cp(n).start()
            for l in range(2):
                for g in range(4):
                    k_s[l, g, 0:HALO, :] = jnp.zeros((HALO, 128), f32)
                    v_s[l, g, 0:HALO, :] = jnp.zeros((HALO, 128), f32)
            z_s[...] = jnp.zeros((RC, 128), u32)
            lm = lmat()
            wait("x0")
            xa = load_x(0)
            xb = load_x(1)
            na = ln1(xa)
            nb = ln1(xb)
            wait("wq")
            perm_sec(lm, 0)
            q_q(na, 0, 0)
            q_q(nb, 0, 1)
            wait("wk")
            perm_sec(lm, 1)
            q_k(na, 0, 0)
            q_k(nb, 0, 1)
            wait("wv", "wo")
            perm_sec(lm, 2)
            q_v(na, 0, 0)
            perm_wo(lm)
            q_v(nb, 0, 1)
            xa = attn_o(xa, 0, 0, True)
            xb = attn_o(xb, 0, 1, True)
            ya = ln2(xa)
            wait("w1", "b1", "b2")
            w1_p[...] = _pk(w1t_v[...])
            ha = up(ya, raw=True)
            hb = up(ln2(xb))
            wait("w2", "x1")
            w2_p[...] = _pk(w2_v[...])
            xa = down(xa, ha, raw=True)
            xb = down(xb, hb)
            na = ln1(xa)
            q_q(na, 1, 0)
            q_k(na, 1, 0)
            q_v(na, 1, 0)
            nb = ln1(xb)
            q_q(nb, 1, 1)
            q_k(nb, 1, 1)
            xa = attn_o(xa, 1, 0, True)
            q_v(nb, 1, 1)
        else:
            xa = load_x(0)
            na = _upk(xn_s[...])
            q_q(na, 0, 0)
            q_k(na, 0, 0)
            q_v(na, 0, 0)
            xb = load_x(1)
            nb = ln1(xb)
            q_q(nb, 0, 1)
            q_k(nb, 0, 1)
            xa = attn_o(xa, 0, 0, False)
            q_v(nb, 0, 1)
            ha = up(ln2(xa))
            xb = attn_o(xb, 0, 1, False)
            xa = down(xa, ha)
            hb = up(ln2(xb))
            na = ln1(xa)
            q_q(na, 1, 0)
            q_k(na, 1, 0)
            q_v(na, 1, 0)
            xb = down(xb, hb)
            xa = attn_o(xa, 1, 0, False)
            nb = ln1(xb)
            q_q(nb, 1, 1)
            q_k(nb, 1, 1)
            q_v(nb, 1, 1)
        ha = up(ln2(xa))
        xb = attn_o(xb, 1, 1, first)
        xa = down(xa, ha)
        emit(xa, 0)
        hb = up(ln2(xb))
        nxt = T if first else pl.multiple_of(jnp.minimum(step + 1, NSTEP - 1) * T, T)
        xn_s[...] = _pk(ln1(x_v[pl.ds(nxt, R), :].astype(f32)))
        xb = down(xb, hb)
        emit(xb, 1)
        if first:
            wait("xr")

    @pl.when(step == 0)
    def _():
        body(True)

    @pl.when(step > 0)
    def _():
        body(False)

    @pl.when(step == NSTEP - 1)
    def _fin():
        for i in range(NSTEP * 2):
            o_copy(i).wait()


@jax.jit
def pallas_interleave_layers__sliding_local_dilated__mixer_channel_mlp__prompt_kernel(
    A_x, A_wqkv, A_wo, B_x, B_w1, B_b1, B_w2, B_b2,
):
    x = A_x.reshape(S, D)
    w1t = B_w1.T
    hbm = pl.BlockSpec(memory_space=pl.ANY)
    out = pl.pallas_call(
        _kernel,
        grid=(NSTEP,),
        in_specs=[hbm] * 7,
        out_specs=hbm,
        out_shape=jax.ShapeDtypeStruct((S, D), A_x.dtype),
        scratch_shapes=[
            pltpu.VMEM((S, D), bf16),
            pltpu.VMEM((S, D), bf16),
            pltpu.VMEM((D, 3 * D), bf16),
            pltpu.VMEM((D, D), bf16),
            pltpu.VMEM((F, D), bf16),
            pltpu.VMEM((F,), bf16),
            pltpu.VMEM((F, D), bf16),
            pltpu.VMEM((D,), bf16),
            pltpu.VMEM((3, D // 2, D), u32),
            pltpu.VMEM((D // 2, D), u32),
            pltpu.VMEM((F // 2, D), u32),
            pltpu.VMEM((F // 2, D), u32),
            pltpu.VMEM((R // 2, D), u32),
            pltpu.VMEM((4, T, 128), f32),
            pltpu.VMEM((2, 4, T + HALO, 128), f32),
            pltpu.VMEM((2, 4, T + HALO, 128), f32),
            pltpu.VMEM((RC, 128), u32),
            pltpu.SemaphoreType.DMA((11,)),
            pltpu.SemaphoreType.DMA((NSTEP * 2,)),
        ],
        compiler_params=pltpu.CompilerParams(
            dimension_semantics=("arbitrary",),
            vmem_limit_bytes=100 * 1024 * 1024,
        ),
    )(x, A_wqkv, A_wo, w1t, B_b1, B_w2, B_b2)
    return out.reshape(1, S, D)
```

```python
import math

import jax
import jax.numpy as jnp
import jax.experimental.pallas as pl
import jax.experimental.pallas.tpu as pltpu

S, D, F = 2048, 512, 1376
H, DH, W, DIL = 32, 16, 8, 2
EPS = 1e-5
HALO = 16
B0 = (128, 128)
BL = (112, 112, 112, 112)
RC = 8
FM = 1280
UP_SPLIT = 6 * 128
GATE = {True: (2, 2), False: (2, 2)}
ORDER = ("Qa0 qb0 kb0 Oa0 vb0 Ua Ob0 Da Ub Qa1 Db Oa1 Qb1 Ua Ob1 Ea Ub "
         "Qc0 Eb qd0 Oc0 kd0 vd0 Uc Od0 Dc Ud Qc1 Dd Oc1 Qd1 Uc Od1 Ec Ud L Ed")
T0, TL = sum(B0), sum(BL)
NSTEP = 1 + (S - T0) // TL
assert T0 + (NSTEP - 1) * TL == S
TM = max(T0, TL)

f32, bf16, u32 = jnp.float32, jnp.bfloat16, jnp.uint32
NT = (((1,), (1,)), ((), ()))
LOG2E = math.log2(math.e)
QSCALE = (DH ** -0.5) * LOG2E
MASKED = -1e9 * LOG2E
GELU_C1 = math.sqrt(2.0 / math.pi)
GELU_C2 = GELU_C1 * 0.044715


def _ln_stats(x):
    m = jnp.mean(x, axis=-1, keepdims=True)
    xc = x - m
    return xc, jnp.mean(xc * xc, axis=-1, keepdims=True)


def _ln1(x):
    xc, v = _ln_stats(x)
    return (xc * jax.lax.rsqrt(v + EPS)).astype(bf16)


def _ln2(x):
    xc, v = _ln_stats(x)
    return (xc * jax.lax.rsqrt(v * (1.0 + EPS) + EPS * EPS)).astype(bf16)


def _pk(x):
    return pltpu.bitcast(x, u32)


def _upk(x):
    return pltpu.bitcast(x, bf16)


def _kernel(x_hbm, wqkv_hbm, wo_hbm, w1t_hbm, b1_hbm, w2_hbm, b2_hbm, o_hbm,
            x_v, o_v, wqkv_v, wo_v, w1t_v, b1_v, w2_v, b2_v,
            wt_p, wo_p, w1_p, w2_p, xn_s, q_s, k_s, v_s, z_s, in_sem, o_sem):
    step = pl.program_id(0)

    copies = {}

    def add_copy(name, src, dst):
        copies[name] = (src, dst, len(copies))

    def rows_copy(name, r0, n):
        add_copy(name, x_hbm.at[pl.ds(r0, n), :], x_v.at[pl.ds(r0, n), :])

    def cols_copy(name, c0, n):
        add_copy(name, wqkv_hbm.at[:, pl.ds(c0, n)], wqkv_v.at[:, pl.ds(c0, n)])

    rows_copy("x0", 0, T0)
    cols_copy("wq0", 0, D // 2)
    cols_copy("wq1", D // 2, D // 2)
    cols_copy("wk", D, D)
    cols_copy("wv", 2 * D, D)
    add_copy("wo", wo_hbm, wo_v)
    add_copy("w1", w1t_hbm, w1t_v)
    add_copy("b1", b1_hbm, b1_v)
    add_copy("b2", b2_hbm, b2_v)
    add_copy("w2", w2_hbm, w2_v)
    rows_copy("x1", T0, BL[0])
    rows_copy("xr", T0 + BL[0], S - T0 - BL[0])

    def cp(name):
        src, dst, i = copies[name]
        return pltpu.make_async_copy(src, dst, in_sem.at[i])

    def wait(*names):
        for n in names:
            cp(n).wait()

    def lmat():
        i = jax.lax.broadcasted_iota(jnp.int32, (128, 128), 0)
        j = jax.lax.broadcasted_iota(jnp.int32, (128, 128), 1)
        return jnp.where(((i >> 3) == (j & 15)) & ((i & 7) == (j >> 4)), 1.0, 0.0).astype(bf16)

    def regroup(outs):
        return jnp.concatenate([outs[hh][d * 8:(d + 1) * 8] for d in range(DH) for hh in range(4)], axis=0)

    def perm_tile(lm, t, hh):
        return jax.lax.dot_general(lm, wqkv_v[:, t * D + hh * 128:t * D + (hh + 1) * 128], NT,
                                   preferred_element_type=f32)

    def perm_sec(lm, t, outs=()):
        outs = list(outs) + [perm_tile(lm, t, hh) for hh in range(len(outs), 4)]
        wt_p[t] = _pk(regroup(outs).astype(bf16))

    def perm_wo(lm):
        outs = [jnp.dot(lm, wo_v[hh * 128:(hh + 1) * 128, :], preferred_element_type=f32) for hh in range(4)]
        wo_p[...] = _pk(regroup(outs).astype(bf16))

    def gate(val, dep):
        dz = pltpu.bitcast(dep, u32) & z_s[...]
        return pltpu.bitcast(pltpu.bitcast(val, u32) | dz, val.dtype)

    def up(y, raw=False):
        def wrows(r0, r1):
            return w1t_v[r0:r1, :] if raw else _upk(w1_p[r0 // 2:r1 // 2, :])

        b1 = b1_v[...].astype(f32).reshape(1, F)
        h0 = jax.lax.dot_general(y, wrows(0, UP_SPLIT), NT, preferred_element_type=f32)
        hr = jax.lax.dot_general(wrows(FM, F), y, NT, preferred_element_type=f32)
        h1 = jax.lax.dot_general(y, wrows(UP_SPLIT, FM), NT, preferred_element_type=f32)
        h = jnp.concatenate([h0, h1, hr.T], axis=1) + b1
        t = jnp.tanh(h * (GELU_C1 + GELU_C2 * (h * h)))
        return (h + h * t).astype(bf16)

    def down(x, h, raw=False):
        b2 = b2_v[...].astype(f32).reshape(1, D)
        w = w2_v[...] if raw else _upk(w2_p[...])
        return (x + b2) + 0.5 * jnp.dot(h, w, preferred_element_type=f32)

    def oproj(x, a):
        return x + jnp.dot(a, _upk(wo_p[...]), preferred_element_type=f32)

    def body(first):
        sizes = B0 if first else BL
        offs = [sum(sizes[:i]) for i in range(len(sizes))]
        nb, T = len(sizes), sum(sizes)
        base = 0 if first else pl.multiple_of(T0 + (step - 1) * TL, 16)

        def proj(xn, t, l, s, g0=0, g1=4):
            r0, r1 = offs[s], offs[s] + sizes[s]
            y = jax.lax.dot_general(xn, _upk(wt_p[t, g0 * 64:g1 * 64, :]), NT, preferred_element_type=f32)
            for g in range(g0, g1):
                yg = y[:, (g - g0) * 128:(g - g0 + 1) * 128]
                if t == 0:
                    q_s[g, r0:r1, :] = yg * QSCALE
                elif t == 1:
                    k_s[l, g, HALO + r0:HALO + r1, :] = yg
                else:
                    v_s[l, g, HALO + r0:HALO + r1, :] = yg

        def qkv(xn, l, s):
            for t in range(3):
                proj(xn, t, l, s)

        def attn(l, s, gated=True):
            gd, gsrc = GATE[first]
            nc = sizes[s] // RC
            ps = []
            for c in range(nc):
                r0 = offs[s] + c * RC
                q = [q_s[g, r0:r0 + RC, :] for g in range(4)]
                for w in range(W):
                    off = HALO + r0 - DIL * w
                    p = q[0] * k_s[l, 0, off:off + RC, :]
                    for g in range(1, 4):
                        p = p + q[g] * k_s[l, g, off:off + RC, :]
                    ps.append((p, pltpu.roll(p, 64, 1)))
            ps = [p + r for p, r in ps]
            ps = [(p, pltpu.roll(p, 32, 1)) for p in ps]
            ps = [p + r for p, r in ps]
            rows, deps = [], []
            for c in range(nc):
                r0 = offs[s] + c * RC
                logits = ps[c * W:(c + 1) * W]
                if first:
                    pos = r0 + jax.lax.broadcasted_iota(jnp.int32, (RC, 128), 0)
                    logits = [jnp.where(pos >= DIL * w, p, MASKED) if r0 < DIL * w else p
                              for w, p in enumerate(logits)]
                mm = list(logits)
                while len(mm) > 1:
                    mm = [jnp.maximum(mm[i], mm[i + 1]) for i in range(0, len(mm), 2)]
                m = mm[0]
                if gated and c >= gd:
                    m = gate(m, deps[c - gd])
                e = [jnp.exp2(lg - m) for lg in logits]
                den = e[0]
                for w in range(1, W):
                    den = den + e[w]
                inv = pl.reciprocal(den, approx=True)
                cols, accs = [], []
                for g in range(4):
                    acc = None
                    for w in range(W):
                        off = HALO + r0 - DIL * w
                        t = e[w] * v_s[l, g, off:off + RC, :]
                        acc = t if acc is None else acc + t
                    accs.append(acc)
                    cols.append(acc * inv)
                deps.append((accs + [inv])[gsrc])
                rows.append(jnp.concatenate(cols, axis=1))
            if s == nb - 1:
                for g in range(4):
                    k_s[l, g, 0:HALO, :] = k_s[l, g, T:T + HALO, :]
                    v_s[l, g, 0:HALO, :] = v_s[l, g, T:T + HALO, :]
            return jnp.concatenate(rows, axis=0).astype(bf16)

        def load_x(s):
            return x_v[pl.ds(base + offs[s], sizes[s]), :].astype(f32)

        def emit(x, s):
            rows = pl.ds(base + offs[s], sizes[s])
            o_v[rows, :] = x.astype(bf16)
            pltpu.make_async_copy(o_v.at[rows, :], o_hbm.at[rows, :], o_sem).start()

        def prefetch_ln():
            nxt = T0 if first else pl.multiple_of(T0 + jnp.minimum(step, NSTEP - 2) * TL, 16)
            xn_s[...] = _pk(_ln1(x_v[pl.ds(nxt, BL[0]), :].astype(f32)))

        if first:
            for n in copies:
                cp(n).start()
            for l in range(2):
                for g in range(4):
                    k_s[l, g, 0:HALO, :] = jnp.zeros((HALO, 128), f32)
                    v_s[l, g, 0:HALO, :] = jnp.zeros((HALO, 128), f32)
            z_s[...] = jnp.zeros((RC, 128), u32)
            lm = lmat()
            wait("x0")
            xa = load_x(0)
            xb = load_x(1)
            na = _ln1(xa)
            nb_ = _ln1(xb)
            wait("wq0")
            outs = [perm_tile(lm, 0, hh) for hh in range(2)]
            wait("wq1")
            perm_sec(lm, 0, outs)
            proj(na, 0, 0, 0)
            proj(nb_, 0, 0, 1, 0, 2)
            wait("wk")
            perm_sec(lm, 1)
            proj(nb_, 0, 0, 1, 2, 4)
            proj(na, 1, 0, 0)
            proj(nb_, 1, 0, 1)
            wait("wv", "wo")
            perm_sec(lm, 2)
            perm_wo(lm)
            proj(na, 2, 0, 0)
            proj(nb_, 2, 0, 1)
            xa = oproj(xa, attn(0, 0, gated=False))
            ab = attn(0, 1, gated=False)
            wait("w1", "b1", "b2")
            w1_p[...] = _pk(w1t_v[...])
            xb = oproj(xb, ab)
            ha = up(_ln2(xa), raw=True)
            hb = up(_ln2(xb))
            wait("w2", "x1")
            w2_p[...] = _pk(w2_v[...])
            xa = down(xa, ha, raw=True)
            xb = down(xb, hb)
            na = _ln1(xa)
            qkv(na, 1, 0)
            nb_ = _ln1(xb)
            proj(nb_, 0, 1, 1)
            proj(nb_, 1, 1, 1)
            xa = oproj(xa, attn(1, 0))
            proj(nb_, 2, 1, 1)
            ha = up(_ln2(xa))
            xb = oproj(xb, attn(1, 1))
            xa = down(xa, ha)
            emit(xa, 0)
            hb = up(_ln2(xb))
            prefetch_ln()
            xb = down(xb, hb)
            emit(xb, 1)
            wait("xr")
        else:
            xs, hs, ns = [None] * nb, [None] * nb, {}
            for ph in ORDER.split():
                if ph == "L":
                    prefetch_ln()
                    continue
                s = "abcd".index(ph[1])
                if xs[s] is None:
                    xs[s] = load_x(s)
                if ph[0] in "qkvQ":
                    l = int(ph[2])
                    if (s, l) not in ns:
                        ns[s, l] = _upk(xn_s[...]) if (s, l) == (0, 0) else _ln1(xs[s])
                    if ph[0] == "Q":
                        qkv(ns[s, l], l, s)
                    else:
                        proj(ns[s, l], "qkv".index(ph[0]), l, s)
                elif ph[0] == "O":
                    xs[s] = oproj(xs[s], attn(int(ph[2]), s))
                elif ph[0] == "U":
                    hs[s] = up(_ln2(xs[s]))
                else:
                    xs[s] = down(xs[s], hs[s])
                    if ph[0] == "E":
                        emit(xs[s], s)

    @pl.when(step == 0)
    def _():
        body(True)

    @pl.when(step > 0)
    def _():
        body(False)

    @pl.when(step == NSTEP - 1)
    def _():
        pltpu.make_async_copy(o_v, o_hbm, o_sem).wait()


@jax.jit
def pallas_interleave_layers__sliding_local_dilated__mixer_channel_mlp__prompt_kernel(
    A_x: jax.Array,
    A_wqkv: jax.Array,
    A_wo: jax.Array,
    B_x: jax.Array,
    B_w1: jax.Array,
    B_b1: jax.Array,
    B_w2: jax.Array,
    B_b2: jax.Array,
):
    del B_x
    hbm = pl.BlockSpec(memory_space=pl.ANY)
    out = pl.pallas_call(
        _kernel,
        grid=(NSTEP,),
        in_specs=[hbm] * 7,
        out_specs=hbm,
        out_shape=jax.ShapeDtypeStruct((S, D), A_x.dtype),
        scratch_shapes=[
            pltpu.VMEM((S, D), bf16),
            pltpu.VMEM((S, D), bf16),
            pltpu.VMEM((D, 3 * D), bf16),
            pltpu.VMEM((D, D), bf16),
            pltpu.VMEM((F, D), bf16),
            pltpu.VMEM((F,), bf16),
            pltpu.VMEM((F, D), bf16),
            pltpu.VMEM((D,), bf16),
            pltpu.VMEM((3, D // 2, D), u32),
            pltpu.VMEM((D // 2, D), u32),
            pltpu.VMEM((F // 2, D), u32),
            pltpu.VMEM((F // 2, D), u32),
            pltpu.VMEM((BL[0] // 2, D), u32),
            pltpu.VMEM((4, TM, 128), f32),
            pltpu.VMEM((2, 4, TM + HALO, 128), f32),
            pltpu.VMEM((2, 4, TM + HALO, 128), f32),
            pltpu.VMEM((RC, 128), u32),
            pltpu.SemaphoreType.DMA((12,)),
            pltpu.SemaphoreType.DMA(()),
        ],
        compiler_params=pltpu.CompilerParams(
            dimension_semantics=("arbitrary",),
            vmem_limit_bytes=64 * 1024 * 1024,
            disable_bounds_checks=True,
            disable_semaphore_checks=True,
        ),
    )(A_x.reshape(S, D), A_wqkv, A_wo, B_w1.T, B_b1, B_w2, B_b2)
    return out.reshape(1, S, D)
```
